```python
import jax
import jax.numpy as jnp

def _softmax(x, axis=-1):
    return jax.nn.softmax(x, axis=axis)

def _gelu(x):
    return jax.nn.gelu(x, approximate=True)

def _silu(x):
    return jax.nn.silu(x)

def _sigmoid(x):
    return jax.nn.sigmoid(x)

def _layernorm(x, axis=-1, eps=1e-05):
    m = jnp.mean(x, axis=axis, keepdims=True)
    v = jnp.var(x, axis=axis, keepdims=True)
    return (x - m) / jnp.sqrt(v + eps)

def _scatter_add(tgt, idx, src, axis=0):
    return tgt.at[idx].add(src)

def _segment_sum(src, seg, n):
    return jax.ops.segment_sum(src, seg, n)

class _Rng:

    def __init__(self, key):
        self._k = key

    def _next(self):
        self._k, sub = jax.random.split(self._k)
        return sub

    def normal(self, shape):
        return jax.random.normal(self._next(), shape, dtype=jnp.bfloat16)

    def randint(self, lo, hi, shape):
        return jax.random.randint(self._next(), shape, lo, hi, dtype=jnp.int32)

    def uniform(self, shape, lo=0.0, hi=1.0):
        return jax.random.uniform(self._next(), shape, jnp.bfloat16, lo, hi)

    def permutation(self, n):
        return jax.random.permutation(self._next(), n)
kernel_name = 'adaLN_cond__sliding_block_cached__moe_arch_mod__decode'

def setup_inputs():
    _rng = _Rng(jax.random.key(int.from_bytes(__import__("os").urandom(4), "little")))
    _w = lambda a: (lambda t: t.astype(jnp.bfloat16) if jnp.issubdtype(t.dtype, jnp.floating) else t)(jnp.asarray(a))

    def _A_setup():
        B, Sq, D = (8, 1, 576)
        Hq, Hkv, Sk, Dh = (32, 16, 8192, 128)
        assert Hq % Hkv == 0, (Hq, Hkv)
        return {'x': _w((lambda *s: _rng.normal(s) * 0.05)(B, Sq, D)), 'k_cache': _w((lambda *s: _rng.normal(s) * 0.05)(B, Hkv, Sk, Dh)), 'v_cache': _w((lambda *s: _rng.normal(s) * 0.05)(B, Hkv, Sk, Dh)), 'wq': _w((lambda *s: _rng.normal(s) * 0.05)(D, Hq * Dh) * D ** (-0.5)), 'wo': _w((lambda *s: _rng.normal(s) * 0.05)(Hq * Dh, D) * (Hq * Dh) ** (-0.5))}
    _A_in = _A_setup()

    def _B_setup():
        B, S, D, F, C = (8, 1, 576, 4608, 1)
        return {'x': _w((lambda *s: _rng.normal(s) * 0.05)(B, S, D)), 'w_r': _w((lambda *s: _rng.normal(s) * 0.05)(D)), 'w_gate': _w((lambda *s: _rng.normal(s) * 0.05)(D, F)), 'w_up': _w((lambda *s: _rng.normal(s) * 0.05)(D, F)), 'w_down': _w((lambda *s: _rng.normal(s) * 0.05)(F, D))}
    _B_in = _B_setup()
    return {'A_x': _A_in['x'], 'A_k_cache': _A_in['k_cache'], 'A_v_cache': _A_in['v_cache'], 'A_wq': _A_in['wq'], 'A_wo': _A_in['wo'], 'B_x': _B_in['x'], 'B_w_r': _B_in['w_r'], 'B_w_gate': _B_in['w_gate'], 'B_w_up': _B_in['w_up'], 'B_w_down': _B_in['w_down'], 'c': _w((lambda *s: _rng.normal(s) * 0.05)(8, 576)), 'w_mod': _w((lambda *s: _rng.normal(s) * 0.05)(576, 6 * 576) * 576 ** (-0.5))}

def reference(A_x, A_k_cache, A_v_cache, A_wq, A_wo, B_x, B_w_r, B_w_gate, B_w_up, B_w_down, c, w_mod):

    def _A_ref(x, k_cache, v_cache, wq, wo):
        B, Sq, D = x.shape
        Hq, Dh = (32, 128)
        Hkv, Sk = (k_cache.shape[1], k_cache.shape[2])
        W = min(4096, max(256, Sk // 4))
        rep = Hq // Hkv
        q = (lambda x, *d: x.transpose(*d))((x @ wq).reshape(B, Sq, Hq, Dh), 0, 2, 1, 3)
        k = jnp.repeat(k_cache[:, :, Sk - W:, :], rep, axis=1)
        v = jnp.repeat(v_cache[:, :, Sk - W:, :], rep, axis=1)
        scores = jnp.einsum('bhqd,bhkd->bhqk', q, k) * Dh ** (-0.5)
        p = _softmax(scores, axis=-1)
        o = jnp.einsum('bhqk,bhkd->bhqd', p, v)
        return (lambda x, *d: x.transpose(*d))(o, 0, 2, 1, 3).reshape(B, Sq, Hq * Dh) @ wo

    def _B_ref(x, w_r, w_gate, w_up, w_down):
        B, S, D = x.shape
        C = 1
        r = x @ w_r
        idx = jnp.argsort(-r, axis=-1)[:, :C]
        idx_e = jnp.repeat(idx.reshape(B, C, 1), D, axis=2)
        x_sel = jnp.take_along_axis(x, idx_e, axis=1)
        g = _silu(x_sel @ w_gate)
        u = x_sel @ w_up
        y = g * u @ w_down
        r_sel = _sigmoid(jnp.take_along_axis(r, idx, axis=1))
        y = y * r_sel.reshape(B, C, 1)
        b_off = (jnp.arange(B) * S).reshape(B, 1)
        flat_idx = (idx + b_off).reshape(B * C)
        zero = (x * 0.0).reshape(B * S, D)
        upd = _scatter_add(zero, flat_idx, y.reshape(B * C, D), axis=0)
        return x + upd.reshape(B, S, D)
    x = A_x
    mod = (_silu(c) @ w_mod).reshape(c.shape[0], 6, 1, -1)
    sa, ca, ga, sb, cb, gb = (mod[:, 0].copy(), mod[:, 1].copy(), mod[:, 2].copy(), mod[:, 3].copy(), mod[:, 4].copy(), mod[:, 5].copy())
    h = _layernorm(x, axis=-1) * (1 + ca) + sa
    x = x + ga * _A_ref(h, A_k_cache, A_v_cache, A_wq, A_wo)
    h = _layernorm(x, axis=-1) * (1 + cb) + sb
    x = x + gb * _B_ref(h, B_w_r, B_w_gate, B_w_up, B_w_down)
    return x
```

```python
import jax
import jax.numpy as jnp
from jax import lax
from jax.experimental import pallas as pl
from jax.experimental.pallas import tpu as pltpu

F32 = jnp.float32
BF16 = jnp.bfloat16
NT = (((1,), (1,)), ((), ()))


def _layernorm(x):
    m = jnp.mean(x, axis=-1, keepdims=True)
    d = x - m
    v = jnp.mean(d * d, axis=-1, keepdims=True)
    return d / jnp.sqrt(v + 1e-5)


def make(nh=4, rows=32, G=4, wr_=16, wc_=1024, kvmode="kv", do_compute=True, unroll_pairs=True, do_dma=True):
    def kernel(x_hbm, k_hbm, v_hbm, wq_hbm, wo_hbm, wr_hbm, wg_hbm, wu_hbm, wd_hbm, c_hbm, wm_hbm,
               o_ref,
               x_v, c_v, wr_v, wm_v, wq_v, wo_v, wg_v, wu_v, wd_v, kv_v, q_s, o_s,
               sem_small, sem_w, sem_kv):
        B, D = x_v.shape
        _, HKV, SK, DH = k_hbm.shape
        W = kv_v.shape[3]
        L = G - 1
        HG = HKV // nh
        NG = B * HG
        row_chunks = [(r, min(128, D - r)) for r in range(0, D, 128)]
        NC = len(row_chunks)

        def small_copies():
            return [pltpu.make_async_copy(s, d, sem_small.at[i])
                    for i, (s, d) in enumerate(((c_hbm, c_v), (x_hbm, x_v), (wr_hbm, wr_v)))]

        weights = [(wm_hbm, wm_v), (wq_hbm, wq_v), (wo_hbm, wo_v), (wg_hbm, wg_v), (wu_hbm, wu_v), (wd_hbm, wd_v)]
        WM, WQ, WO, WG, WU, WD = range(6)

        def start_w(w, ci):
            if not do_dma:
                return
            src, dst = weights[w]
            r0, nr = row_chunks[ci]
            ncol = src.shape[1]
            npc = -(-ncol // wc_)
            if npc % 2:
                npc += 1
            tiles = ncol // 128
            bounds = [(tiles * i // npc) * 128 for i in range(npc + 1)]

            def body(i, _):
                r = pl.multiple_of(r0 + i * wr_, wr_)
                for j in range(npc):
                    cs = pl.ds(bounds[j], bounds[j + 1] - bounds[j])
                    pltpu.make_async_copy(src.at[pl.ds(r, wr_), cs], dst.at[pl.ds(r, wr_), cs],
                                          sem_w.at[w * NC + ci]).start(priority=j % 2)
                return 0
            lax.fori_loop(0, nr // wr_, body, 0)

        def wait_w(w, ci):
            if not do_dma:
                return
            _, dst = weights[w]
            r0, nr = row_chunks[ci]
            d = dst.at[pl.ds(r0, nr), :]
            pltpu.make_async_copy(d, d, sem_w.at[w * NC + ci]).wait()

        part = W // nh

        def start_kv(g, j):
            if not do_dma:
                return
            slot = g % G
            b = g // HG
            h0 = (g % HG) * nh

            def body(i, _):
                r = pl.multiple_of(j * part + i * rows, rows)
                for w, src in enumerate((k_hbm, v_hbm)):
                    pltpu.make_async_copy(src.at[b, pl.ds(h0, nh), pl.ds(SK - W + r, rows), :],
                                          kv_v.at[slot, w, :, pl.ds(r, rows), :],
                                          sem_kv.at[slot]).start(priority=w)
                return 0
            lax.fori_loop(0, part // rows, body, 0, unroll=4)

        def wait_kv(g):
            if not do_dma:
                return
            slot = g % G
            pltpu.make_async_copy(kv_v.at[slot], kv_v.at[slot], sem_kv.at[slot]).wait()

        head = [(WM, ci) for ci in range(NC)] + [(WQ, ci) for ci in range(NC)]
        tail = ([(WO, ci) for ci in range(NC)]
                + [(w, ci) for ci in range(NC) for w in (WG, WU)]
                + [(WD, ci) for ci in range(NC)])
        LOOK = L * nh
        n_head, n_kv, n_tail = len(head), NG * nh, len(tail)

        def start_static(t):
            if t < n_head:
                start_w(*head[t])
            elif t < n_head + n_kv:
                start_kv((t - n_head) // nh, (t - n_head) % nh)
            elif t < n_head + n_kv + n_tail:
                start_w(*tail[t - n_head - n_kv])

        for cp in small_copies():
            cp.start()
        PRE = 5
        for t in range(PRE):
            start_static(t)
        nxt = PRE
        per_step = -(-(n_head + LOOK - PRE) // n_head)

        def issue_more(nxt, limit):
            for _ in range(per_step):
                if nxt < limit:
                    start_static(nxt)
                    nxt += 1
            return nxt

        for cp in small_copies():
            cp.wait()
        cf = c_v[...].astype(F32)
        sc = (cf * jax.nn.sigmoid(cf)).astype(BF16)
        mod = None
        for ci, (r0, nr) in enumerate(row_chunks):
            wait_w(WM, ci)
            p = jnp.dot(sc[:, r0:r0 + nr], wm_v[r0:r0 + nr, :], preferred_element_type=F32)
            mod = p if mod is None else mod + p
            nxt = issue_more(nxt, n_head + LOOK)
        sa, ca, ga, sb, cb, gb = (mod[:, i * D:(i + 1) * D] for i in range(6))
        x = x_v[...].astype(F32)
        h = (_layernorm(x) * (1.0 + ca) + sa).astype(BF16)
        q = None
        for ci, (r0, nr) in enumerate(row_chunks):
            wait_w(WQ, ci)
            p = jnp.dot(h[:, r0:r0 + nr], wq_v[r0:r0 + nr, :], preferred_element_type=F32)
            q = p if q is None else q + p
            nxt = issue_more(nxt, n_head + LOOK)
        assert nxt == n_head + LOOK
        for hk in range(HKV):
            q2 = jnp.concatenate([q[:, (2 * hk) * DH:(2 * hk + 1) * DH],
                                  q[:, (2 * hk + 1) * DH:(2 * hk + 2) * DH]], axis=0)
            q_s[hk] = q2.astype(BF16)
        o_s[...] = jnp.zeros_like(o_s)

        scale = DH ** -0.5
        row_b = lax.broadcasted_iota(jnp.int32, (2 * B, DH), 0) % B

        def attend(g, j):
            if not do_compute:
                return
            slot = g % G
            b = g // HG
            hk = (g % HG) * nh + j
            s = lax.dot_general(q_s[hk], kv_v[slot, 0, j], NT, preferred_element_type=F32) * scale
            m = jnp.max(s, axis=-1, keepdims=True)
            p = jnp.exp(s - m)
            l = jnp.sum(p, axis=-1, keepdims=True)
            o = jnp.dot(p.astype(BF16), kv_v[slot, 1, j], preferred_element_type=F32) / l
            o_s[hk] = jnp.where(row_b == b, o, o_s[hk])

        def group(g, _):
            wait_kv(g)
            if unroll_pairs:
                for j in range(nh):
                    attend(g, j)
                    start_kv(g + L, j)
            else:
                def pair(j, _):
                    attend(g, j)
                    start_kv(g + L, j)
                    return 0
                lax.fori_loop(0, nh, pair, 0)
            return 0
        lax.fori_loop(0, NG - L, group, 0)

        nxt = n_head + n_kv
        total = n_head + n_kv + n_tail
        for g in range(NG - L, NG):
            wait_kv(g)
            for j in range(nh):
                attend(g, j)
                if nxt < total:
                    start_static(nxt)
                    nxt += 1

        def issue_one(nxt):
            if nxt < total:
                start_static(nxt)
                nxt += 1
            return nxt

        o = jnp.concatenate([o_s[hk, i * B:(i + 1) * B, :] for hk in range(HKV) for i in range(2)],
                            axis=1).astype(BF16)
        parts = []
        for ci, (r0, nr) in enumerate(row_chunks):
            wait_w(WO, ci)
            parts.append(lax.dot_general(o, wo_v[r0:r0 + nr, :], NT, preferred_element_type=F32))
            nxt = issue_one(nxt)
        x1 = x + ga * jnp.concatenate(parts, axis=1)
        h2 = _layernorm(x1) * (1.0 + cb) + sb
        r = jnp.sum(h2 * wr_v[...].astype(F32).reshape(1, D), axis=-1, keepdims=True)
        h2b = h2.astype(BF16)
        gate = up = None
        for ci, (r0, nr) in enumerate(row_chunks):
            wait_w(WG, ci)
            p = jnp.dot(h2b[:, r0:r0 + nr], wg_v[r0:r0 + nr, :], preferred_element_type=F32)
            gate = p if gate is None else gate + p
            nxt = issue_one(nxt)
            wait_w(WU, ci)
            p = jnp.dot(h2b[:, r0:r0 + nr], wu_v[r0:r0 + nr, :], preferred_element_type=F32)
            up = p if up is None else up + p
            nxt = issue_one(nxt)
        act = (gate * jax.nn.sigmoid(gate) * up).astype(BF16)
        rs = jax.nn.sigmoid(r)
        for ci, (r0, nr) in enumerate(row_chunks):
            nxt = issue_one(nxt)
            wait_w(WD, ci)
            y = lax.dot_general(act, wd_v[r0:r0 + nr, :], NT, preferred_element_type=F32)
            cs = slice(r0, r0 + nr)
            hh = h2[:, cs]
            o_ref[:, cs] = (x1[:, cs] + gb[:, cs] * (hh + (hh * 0.0 + y * rs))).astype(o_ref.dtype)
        assert nxt == total

    def fn(A_x, A_k_cache, A_v_cache, A_wq, A_wo, B_x, B_w_r, B_w_gate, B_w_up, B_w_down, c, w_mod):
        B, _, D = A_x.shape
        _, HKV, SK, DH = A_k_cache.shape
        W = min(4096, max(256, SK // 4))
        HD = A_wq.shape[1]
        F = B_w_gate.shape[1]
        hbm = pl.BlockSpec(memory_space=pltpu.HBM)
        out = pl.pallas_call(
            kernel,
            out_shape=jax.ShapeDtypeStruct((B, D), A_x.dtype),
            in_specs=[hbm] * 11,
            out_specs=pl.BlockSpec(memory_space=pltpu.VMEM),
            scratch_shapes=[
                pltpu.VMEM((B, D), BF16), pltpu.VMEM((B, D), BF16), pltpu.VMEM((D,), BF16),
                pltpu.VMEM((D, 6 * D), BF16), pltpu.VMEM((D, HD), BF16), pltpu.VMEM((D, HD), BF16),
                pltpu.VMEM((D, F), BF16), pltpu.VMEM((D, F), BF16), pltpu.VMEM((D, F), BF16),
                pltpu.VMEM((G, 2, nh, W, DH), BF16),
                pltpu.VMEM((HKV, 2 * B, DH), BF16), pltpu.VMEM((HKV, 2 * B, DH), F32),
                pltpu.SemaphoreType.DMA((3,)), pltpu.SemaphoreType.DMA((30,)), pltpu.SemaphoreType.DMA((G,)),
            ],
            compiler_params=pltpu.CompilerParams(vmem_limit_bytes=100 * 1024 * 1024),
        )(A_x.reshape(B, D), A_k_cache, A_v_cache, A_wq, A_wo.T, B_w_r, B_w_gate, B_w_up, B_w_down.T, c, w_mod)
        return out.reshape(B, 1, D)
    return fn


_impl = make()


@jax.jit
def pallas_adaLN_cond__sliding_block_cached__moe_arch_mod__decode_kernel(
    A_x, A_k_cache, A_v_cache, A_wq, A_wo, B_x, B_w_r, B_w_gate, B_w_up, B_w_down, c, w_mod,
):
    return _impl(A_x, A_k_cache, A_v_cache, A_wq, A_wo, B_x, B_w_r, B_w_gate, B_w_up, B_w_down, c, w_mod)
```

```python
import jax
import jax.numpy as jnp
from jax import lax
from jax.experimental import pallas as pl
from jax.experimental.pallas import tpu as pltpu

F32 = jnp.float32
BF16 = jnp.bfloat16
NT = (((1,), (1,)), ((), ()))


def _layernorm(x):
    m = jnp.mean(x, axis=-1, keepdims=True)
    d = x - m
    v = jnp.mean(d * d, axis=-1, keepdims=True)
    return d / jnp.sqrt(v + 1e-5)


def make(rows=32, G=3, voff=32, nobc=True, do_compute=True, do_tail=True, small_late=False):
    NH = 4
    CW = 512
    P = 4
    PM = 6

    def kernel(x_hbm, k_hbm, v_hbm, wq_hbm, wo_hbm, wr_hbm, wg_hbm, wu_hbm, wd_hbm, c_hbm, wm_hbm,
               o_ref,
               x_v, c_v, wr_v, wm_v, wq_v, wo_v, wg_v, wu_v, wd_v, kv_v, mod_s, q_s, o_s, act_s,
               sem_small, sem_w, sem_d, sem_kv):
        B, D = x_v.shape
        _, HKV, SK, DH = k_hbm.shape
        W = kv_v.shape[3]
        L = G - 1
        HG = HKV // NH
        NG = B * HG
        R = D // P
        NQ = wq_v.shape[0]
        NF = wg_v.shape[0]
        NFA = (NF + 1) // 2
        S_M, S_Q, S_O, S_GA, S_UA, S_GB, S_UB = range(7)

        def small_copies():
            return [pltpu.make_async_copy(s, d, sem_small.at[i])
                    for i, (s, d) in enumerate(((c_hbm, c_v), (x_hbm, x_v), (wr_hbm, wr_v)))]

        def copy_w(src, dst, j, blocks, r, sem, priority):
            cw = dst.shape[-1]
            c0 = j * cw if isinstance(j, int) else pl.multiple_of(j * cw, cw)
            pltpu.make_async_copy(src.at[blocks, pl.ds(r, 8), pl.ds(c0, cw)],
                                  dst.at[j, blocks, pl.ds(r, 8), :], sem).start(priority=priority)

        def wait_buf(buf, sem):
            pltpu.make_async_copy(buf, buf, sem).wait()

        def rows_loop(lo, hi, fn):
            def body(i, _):
                fn(pl.multiple_of(i * 8, 8))
                return 0
            lax.fori_loop(lo, hi, body, 0)

        def start_mod():
            def step(r):
                for j in range(wm_v.shape[0]):
                    copy_w(wm_hbm, wm_v, j, pl.ds(0, PM // 2), r, sem_w.at[S_M], 0)
                    copy_w(wm_hbm, wm_v, j, pl.ds(PM // 2, PM // 2), r, sem_w.at[S_M], 1)
            rows_loop(0, D // PM // 8, step)

        def start_pair(a, b, chunks, lo, hi):
            def step(r):
                for j in chunks:
                    copy_w(a[0], a[1], j, pl.ds(0, P), r, sem_w.at[a[2]], 0)
                    copy_w(b[0], b[1], j, pl.ds(0, P), r, sem_w.at[b[2]], 1)
            rows_loop(lo, hi, step)

        def start_qo(u, n=1):
            start_pair((wq_hbm, wq_v, S_Q), (wo_hbm, wo_v, S_O), range(NQ), 2 * u, 2 * (u + n))

        def start_gu_a(u):
            start_pair((wg_hbm, wg_v, S_GA), (wu_hbm, wu_v, S_UA), range(NFA), 3 * u, 3 * u + 3)

        def start_gu_b(u):
            start_pair((wg_hbm, wg_v, S_GB), (wu_hbm, wu_v, S_UB), range(NFA, NF), 3 * u, 3 * u + 3)

        def start_down(j):
            def step(r):
                copy_w(wd_hbm, wd_v, j, pl.ds(0, P), r, sem_d.at[j], 0)
                copy_w(wd_hbm, wd_v, j, pl.ds(0, P), pl.multiple_of(r + R // 2, 8), sem_d.at[j], 1)
            rows_loop(0, R // 16, step)

        nr = W // rows
        part = nr // NH

        def start_kv(t):
            g = t // NH
            slot = g % G
            b = g // HG
            h0 = (g % HG) * NH

            def body(i, _):
                for w, src in enumerate((k_hbm, v_hbm)):
                    r = pl.multiple_of(((i + w * voff) % nr) * rows, rows)
                    pltpu.make_async_copy(src.at[b, pl.ds(h0, NH), pl.ds(SK - W + r, rows), :],
                                          kv_v.at[slot, w, :, pl.ds(r, rows), :],
                                          sem_kv.at[slot]).start(priority=w)
                return 0
            i0 = (t % NH) * part
            lax.fori_loop(0, part, lambda i, c: body(i0 + i, c), 0, unroll=2)

        def kv_loop(lo, hi):
            def body(t, _):
                start_kv(t)
                return 0
            lax.fori_loop(lo, hi, body, 0)

        if not small_late:
            for cp in small_copies():
                cp.start()
        start_mod()
        if small_late:
            for cp in small_copies():
                cp.start()
        start_qo(0, 4)
        for cp in small_copies():
            cp.wait()
        cf = c_v[...].astype(F32)
        sc = (cf * jax.nn.sigmoid(cf)).astype(BF16)
        wait_buf(wm_v, sem_w.at[S_M])

        def mod_step(j, _):
            mod_s[j] = jnp.dot(sc, wm_v[j].reshape(D, 2 * D), preferred_element_type=F32)
            start_qo(4 + j)
            return 0
        lax.fori_loop(0, 3, mod_step, 0)
        x = x_v[...].astype(F32)
        h = (_layernorm(x) * (1.0 + mod_s[0, :, D:]) + mod_s[0, :, :D]).astype(BF16)
        start_qo(7, 2)
        kv_loop(0, 4)
        wait_buf(wq_v, sem_w.at[S_Q])
        n_more = L * NH - 4

        def q_step(j, _):
            q = jnp.dot(h, wq_v[j].reshape(D, CW), preferred_element_type=F32)
            for i in range(2):
                q2 = jnp.concatenate([q[:, (2 * i) * DH:(2 * i + 1) * DH],
                                      q[:, (2 * i + 1) * DH:(2 * i + 2) * DH]], axis=0)
                q_s[2 * j + i] = q2.astype(BF16)
            kv_loop(4 + (j * n_more) // NQ, 4 + ((j + 1) * n_more) // NQ)
            return 0
        lax.fori_loop(0, NQ, q_step, 0)
        o_s[...] = jnp.zeros_like(o_s)

        scale = DH ** -0.5
        row_b = lax.broadcasted_iota(jnp.int32, (2 * B, DH), 0) % B
        NT_ = NG * NH

        def attend(t, _):
            g = t // NH
            j = t % NH
            slot = g % G
            b = g // HG
            hk = (g % HG) * NH + j

            @pl.when(j == 0)
            def _():
                wait_buf(kv_v.at[slot], sem_kv.at[slot])

            if do_compute:
                s = lax.dot_general(q_s[hk], kv_v[slot, 0, j], NT, preferred_element_type=F32) * scale
                m = jnp.max(s, axis=-1, keepdims=True)
                p = jnp.exp(s - m)
                l = jnp.sum(p, axis=-1, keepdims=True)
                o = jnp.dot(p.astype(BF16), kv_v[slot, 1, j], preferred_element_type=F32) / l
                o_s[hk] = jnp.where(row_b == b, o, o_s[hk])
            u = t + L * NH

            @pl.when(u < NT_)
            def _():
                start_kv(u)

            @pl.when(jnp.logical_and(u >= NT_, u < NT_ + 6))
            def _():
                start_gu_a(u - NT_)

            @pl.when(u >= NT_ + 6)
            def _():
                start_gu_b(u - NT_ - 6)
            return 0
        lax.fori_loop(0, NT_, attend, 0)
        gb_done = L * NH - 6
        assert 0 <= gb_done <= 6

        wait_buf(wo_v, sem_w.at[S_O])
        gb_mid = max(gb_done, 4)

        def wo_step(j, acc):
            o = jnp.concatenate([o_s[2 * j + i, k * B:(k + 1) * B, :] for i in range(2) for k in range(2)],
                                axis=1).astype(BF16)
            acc = acc + lax.dot_general(o, wo_v[j].reshape(D, CW), NT, preferred_element_type=F32)
            for n, u in enumerate(range(gb_done, gb_mid)):
                @pl.when(j == 2 + 3 * n)
                def _():
                    start_gu_b(u)
            return acc
        attn = lax.fori_loop(0, NQ, wo_step, jnp.zeros((B, D), F32))
        x1 = x + mod_s[1, :, :D] * attn
        h2 = _layernorm(x1) * (1.0 + mod_s[2, :, :D]) + mod_s[1, :, D:]
        r = jnp.sum(h2 * wr_v[...].astype(F32).reshape(1, D), axis=-1, keepdims=True)
        h2b = h2.astype(BF16)

        def gate_up(j):
            gate = jnp.dot(h2b, wg_v[j].reshape(D, CW), preferred_element_type=F32)
            up = jnp.dot(h2b, wu_v[j].reshape(D, CW), preferred_element_type=F32)
            act_s[j] = gate * jax.nn.sigmoid(gate) * up

        wait_buf(wg_v.at[pl.ds(0, NFA)], sem_w.at[S_GA])
        wait_buf(wu_v.at[pl.ds(0, NFA)], sem_w.at[S_UA])
        n_gb = 6 - gb_mid

        def gu_a_step(j, _):
            gate_up(j)

            @pl.when(j < n_gb)
            def _():
                start_gu_b(gb_mid + j)

            @pl.when(j >= n_gb)
            def _():
                start_down(j - n_gb)
            return 0
        lax.fori_loop(0, NFA, gu_a_step, 0)
        d_done = NFA - n_gb
        d_mid = NF - (NF - NFA - 1)

        def d_body(j, _):
            start_down(j)
            return 0
        lax.fori_loop(d_done, d_mid, d_body, 0)
        wait_buf(wg_v.at[pl.ds(NFA, NF - NFA)], sem_w.at[S_GB])
        wait_buf(wu_v.at[pl.ds(NFA, NF - NFA)], sem_w.at[S_UB])

        def gu_b_step(j, _):
            gate_up(j)

            @pl.when(j < NF - 1)
            def _():
                start_down(j - NFA + d_mid)
            return 0
        lax.fori_loop(NFA, NF, gu_b_step, 0)

        def down_step(j, acc):
            wait_buf(wd_v.at[j], sem_d.at[j])
            if not do_tail:
                return acc
            return acc + lax.dot_general(act_s[j].astype(BF16), wd_v[j].reshape(D, CW), NT,
                                         preferred_element_type=F32)
        y = lax.fori_loop(0, NF, down_step, jnp.zeros((B, D), F32))
        o_ref[...] = (x1 + mod_s[2, :, D:] * (h2 + (h2 * 0.0 + y * jax.nn.sigmoid(r)))).astype(o_ref.dtype)

    def fn(A_x, A_k_cache, A_v_cache, A_wq, A_wo, B_x, B_w_r, B_w_gate, B_w_up, B_w_down, c, w_mod):
        B, _, D = A_x.shape
        _, HKV, SK, DH = A_k_cache.shape
        W = min(4096, max(256, SK // 4))
        HD = A_wq.shape[1]
        F = B_w_gate.shape[1]
        hbm = pl.BlockSpec(memory_space=pltpu.HBM)
        blk = lambda w, p=P: w.reshape(p, D // p, w.shape[1])
        wbuf = lambda n: pltpu.VMEM((n // CW, P, D // P, CW), BF16)
        out = pl.pallas_call(
            kernel,
            out_shape=jax.ShapeDtypeStruct((B, D), A_x.dtype),
            in_specs=[hbm] * 11,
            out_specs=pl.BlockSpec(memory_space=pltpu.VMEM),
            scratch_shapes=[
                pltpu.VMEM((B, D), BF16), pltpu.VMEM((B, D), BF16), pltpu.VMEM((D,), BF16),
                pltpu.VMEM((3, PM, D // PM, 2 * D), BF16), wbuf(HD), wbuf(HD), wbuf(F), wbuf(F), wbuf(F),
                pltpu.VMEM((G, 2, NH, W, DH), BF16),
                pltpu.VMEM((3, B, 2 * D), F32),
                pltpu.VMEM((HKV, 2 * B, DH), BF16), pltpu.VMEM((HKV, 2 * B, DH), F32),
                pltpu.VMEM((F // CW, B, CW), F32),
                pltpu.SemaphoreType.DMA((3,)), pltpu.SemaphoreType.DMA((7,)),
                pltpu.SemaphoreType.DMA((F // CW,)), pltpu.SemaphoreType.DMA((G,)),
            ],
            compiler_params=pltpu.CompilerParams(vmem_limit_bytes=100 * 1024 * 1024,
                                                 disable_bounds_checks=nobc),
        )(A_x.reshape(B, D), A_k_cache, A_v_cache, blk(A_wq), blk(A_wo.T), B_w_r, blk(B_w_gate), blk(B_w_up),
          blk(B_w_down.T), c, blk(w_mod, PM))
        return out.reshape(B, 1, D)
    return fn


_impl = make()


@jax.jit
def pallas_adaLN_cond__sliding_block_cached__moe_arch_mod__decode_kernel(
    A_x, A_k_cache, A_v_cache, A_wq, A_wo, B_x, B_w_r, B_w_gate, B_w_up, B_w_down, c, w_mod,
):
    return _impl(A_x, A_k_cache, A_v_cache, A_wq, A_wo, B_x, B_w_r, B_w_gate, B_w_up, B_w_down, c, w_mod)
```

```python
import jax
import jax.numpy as jnp
from jax import lax
from jax.experimental import pallas as pl
from jax.experimental.pallas import tpu as pltpu

F32 = jnp.float32
BF16 = jnp.bfloat16
NT = (((1,), (1,)), ((), ()))


def _layernorm(x):
    m = jnp.mean(x, axis=-1, keepdims=True)
    d = x - m
    v = jnp.mean(d * d, axis=-1, keepdims=True)
    return d / jnp.sqrt(v + 1e-5)


def make(rows=32, G=3, voff=32, nosc=True, lead=5, esplit=6, pure=False, notail=False, kq=1, dmode=0, scopes=False):
    import contextlib
    ns = (lambda n: jax.named_scope(n)) if scopes else (lambda n: contextlib.nullcontext())
    NH = 4
    CW = 512
    P = 4
    PM = 6

    def kernel(x_hbm, k_hbm, v_hbm, wq_hbm, wo_hbm, wr_hbm, wg_hbm, wu_hbm, wd_hbm, c_hbm, wm_hbm,
               o_ref,
               x_v, c_v, wr_v, wm_v, wq_v, wo_v, wg_v, wu_v, wd_v, kv_v, mod_s, q_s, o_s, act_s, fin_s, y_s,
               sem_w, sem_d, sem_kv):
        B, D = x_v.shape
        _, HKV, SK, DH = k_hbm.shape
        W = kv_v.shape[3]
        L = G - 1
        HG = HKV // NH
        NG = B * HG
        NQ = wq_v.shape[0]
        NF = wg_v.shape[0]
        F = NF * CW
        S_X, S_M, S_Q, S_O, S_G = range(5)

        def small_copies():
            return [pltpu.make_async_copy(s, d, sem_w.at[S_X])
                    for s, d in ((c_hbm, c_v), (x_hbm, x_v), (wr_hbm, wr_v))]

        def copy_w(src, dst, j, blocks, r, sem, priority):
            cw = dst.shape[-1]
            pltpu.make_async_copy(src.at[blocks, pl.ds(r, 8), pl.ds(j * cw, cw)],
                                  dst.at[j, blocks, pl.ds(r, 8), :], sem).start(priority=priority)

        def wait_buf(buf, sem):
            pltpu.make_async_copy(buf, buf, sem).wait()

        def rows_loop(lo, hi, fn):
            def body(i, _):
                fn(pl.multiple_of(i * 8, 8))
                return 0
            lax.fori_loop(lo, hi, body, 0)

        def start_mod(lo, hi, p0):
            def step(r):
                for j in range(wm_v.shape[0]):
                    copy_w(wm_hbm, wm_v, j, pl.ds(0, PM // 2), r, sem_w.at[S_M], p0)
                    copy_w(wm_hbm, wm_v, j, pl.ds(PM // 2, PM // 2), r, sem_w.at[S_M], 1)
            rows_loop(lo, hi, step)

        def start_pair(a, b, lo, hi):
            def step(r):
                for j in range(a[1].shape[0]):
                    copy_w(a[0], a[1], j, pl.ds(0, P), r, sem_w.at[a[2]], 0)
                    copy_w(b[0], b[1], j, pl.ds(0, P), r, sem_w.at[b[2]], 1)
            rows_loop(lo, hi, step)

        def start_qo(u, n=1):
            start_pair((wq_hbm, wq_v, S_Q), (wo_hbm, wo_v, S_O), 2 * u, 2 * (u + n))

        def start_gu(u):
            start_pair((wg_hbm, wg_v, S_G), (wu_hbm, wu_v, S_G), 2 * u, 2 * u + 2)

        DA, DA2, DB, DE0, DE1 = (0, 256), (448, 64), (256, 128), (384, 64), (512, 64)

        def copy_d(rng, r, j, sem, priority):
            r0, n = rng
            src = wd_hbm.at[pl.ds(r0, n)].reshape(P, n // P, F)
            dst = wd_v.at[pl.ds(r0, n)].reshape(P, n // P, F)
            pltpu.make_async_copy(src.at[:, pl.ds(r, 8), pl.ds(j * CW, CW)],
                                  dst.at[:, pl.ds(r, 8), pl.ds(j * CW, CW)], sem).start(priority=priority)

        def start_da(lo, hi, rng=DA, s=0):
            half = rng[1] // P // 2

            def step(r):
                for j in range(NF):
                    copy_d(rng, r, j, sem_d.at[s], 0)
                    copy_d(rng, pl.multiple_of(r + half, 8), j, sem_d.at[s], 1)
            rows_loop(lo, hi, step)

        def start_dlast(i):
            if dmode == 0:
                e_list = [(DE0, r, j, 2) for r in (0, 8) for j in range(NF)]
                e_list += [(DE1, r, j, 3) for r in (0, 8) for j in range(esplit)]
                e_list += [(DE1, r, j, 4) for r in (0, 8) for j in range(esplit, NF)]
            for j in range(NF):
                copy_d(DB, 8 * i, j, sem_d.at[1], 0)
                rng, r, jj, s = e_list[i * NF + j]
                copy_d(rng, r, jj, sem_d.at[s], 1)

        nr = W // rows
        part = nr // NH

        def start_kv(t):
            g = t // NH
            slot = g % G
            b = g // HG
            h0 = (g % HG) * NH

            def body(i, _):
                for w, src in enumerate((k_hbm, v_hbm)):
                    r = pl.multiple_of(((i + w * voff) % nr) * rows, rows)
                    pltpu.make_async_copy(src.at[b, pl.ds(h0, NH), pl.ds(SK - W + r, rows), :],
                                          kv_v.at[slot, w, :, pl.ds(r, rows), :],
                                          sem_kv.at[slot]).start(priority=w ^ kq)
                return 0
            i0 = (t % NH) * part
            lax.fori_loop(0, part, lambda i, c: body(i0 + i, c), 0, unroll=2)

        def kv_loop(lo, hi):
            def body(t, _):
                start_kv(t)
                return 0
            lax.fori_loop(lo, hi, body, 0)

        if lead:
            start_mod(0, lead, 1)
        for cp in small_copies():
            cp.start(priority=1 if lead else 0)
        start_mod(lead, D // PM // 8, 0)
        start_qo(0, 4)
        for cp in small_copies():
            cp.wait()
        cf = c_v[...].astype(F32)
        sc = (cf * jax.nn.sigmoid(cf)).astype(BF16)
        wait_buf(wm_v, sem_w.at[S_M])

        def mod_step(j, _):
            if not pure:
                m = jnp.dot(sc, wm_v[j].reshape(D, 2 * D), preferred_element_type=F32)
                mod_s[2 * j] = m[:, :D]
                mod_s[2 * j + 1] = m[:, D:]
            start_qo(4 + j)
            return 0
        lax.fori_loop(0, 3, mod_step, 0)
        x = x_v[...].astype(F32)
        h = (_layernorm(x) * (1.0 + mod_s[1]) + mod_s[0]).astype(BF16)
        start_qo(7, 2)
        kv_loop(0, 4)
        wait_buf(wq_v, sem_w.at[S_Q])
        n_more = L * NH - 4

        def q_step(j, _):
            if not pure:
                q = jnp.dot(h, wq_v[j].reshape(D, CW), preferred_element_type=F32)
                for i in range(2):
                    q2 = jnp.concatenate([q[:, (2 * i) * DH:(2 * i + 1) * DH],
                                          q[:, (2 * i + 1) * DH:(2 * i + 2) * DH]], axis=0)
                    q_s[2 * j + i] = q2.astype(BF16)
            kv_loop(4 + (j * n_more) // NQ, 4 + ((j + 1) * n_more) // NQ)
            return 0
        lax.fori_loop(0, NQ, q_step, 0)
        o_s[...] = jnp.zeros_like(o_s)

        scale = DH ** -0.5
        row_b = lax.broadcasted_iota(jnp.int32, (2 * B, DH), 0) % B
        NP = NG * NH

        def attend(t, _):
            g = t // NH
            j = t % NH
            slot = g % G
            b = g // HG
            hk = (g % HG) * NH + j

            @pl.when(j == 0)
            def _():
                wait_buf(kv_v.at[slot], sem_kv.at[slot])

            if not pure:
                s = lax.dot_general(q_s[hk], kv_v[slot, 0, j], NT, preferred_element_type=F32) * scale
                m = jnp.max(s, axis=-1, keepdims=True)
                p = jnp.exp(s - m)
                l = jnp.sum(p, axis=-1, keepdims=True)
                o = jnp.dot(p.astype(BF16), kv_v[slot, 1, j], preferred_element_type=F32) / l
                o_s[hk] = jnp.where(row_b == b, o, o_s[hk])
            u = t + L * NH

            @pl.when(u < NP)
            def _():
                start_kv(u)

            @pl.when(u >= NP)
            def _():
                start_gu(u - NP)
            return 0
        with ns('c_att'):
            lax.fori_loop(0, NP, attend, 0)
        assert L * NH == 8

        wait_buf(wo_v, sem_w.at[S_O])

        def wo_step(j, acc):
            if not pure:
                o = jnp.concatenate([o_s[2 * j + i, k * B:(k + 1) * B, :] for i in range(2) for k in range(2)],
                                    axis=1).astype(BF16)
                acc = acc + lax.dot_general(o, wo_v[j].reshape(D, CW), NT, preferred_element_type=F32)

            @pl.when(j == 2)
            def _():
                start_gu(8)

            @pl.when(j == 5)
            def _():
                start_da(0, 1, DA2, 5)
            return acc
        with ns('c_wo'):
            attn = lax.fori_loop(0, NQ, wo_step, jnp.zeros((B, D), F32))
        start_da(0, 1)
        x1 = x + mod_s[2] * attn
        h2 = _layernorm(x1) * (1.0 + mod_s[4]) + mod_s[3]
        r = jnp.sum(h2 * wr_v[...].astype(F32).reshape(1, D), axis=-1, keepdims=True)
        h2b = h2.astype(BF16)
        fin_s[0] = x1 + mod_s[5] * (h2 + h2 * 0.0)
        fin_s[1] = mod_s[5] * jax.nn.sigmoid(r)
        with ns("i_da"):
            start_da(1, 4)
            start_dlast(0)
        with ns("w_g"):
            wait_buf(wg_v, sem_w.at[S_G])
            wait_buf(wu_v, sem_w.at[S_G])

        def gu_step(j, _):
            if not pure:
                gate = jnp.dot(h2b, wg_v[j].reshape(D, CW), preferred_element_type=F32)
                up = jnp.dot(h2b, wu_v[j].reshape(D, CW), preferred_element_type=F32)
                act_s[j] = gate * jax.nn.sigmoid(gate) * up
            for i in range(1, 4):
                @pl.when(j == 2 * i - 1)
                def _():
                    start_dlast(i)
            return 0
        with ns('c_gu'):
            lax.fori_loop(0, NF, gu_step, 0)
        act = jnp.concatenate([act_s[j] for j in range(NF)], axis=1).astype(BF16)

        def down(r0, n, c0=0, c1=F):
            return lax.dot_general(act[:, c0:c1], wd_v[r0:r0 + n, c0:c1], NT, preferred_element_type=F32)

        def finish(r0, y):
            cs = slice(r0, r0 + y.shape[1])
            o_ref[:, cs] = (fin_s[0, :, cs] + fin_s[1, :, cs] * y).astype(o_ref.dtype)

        with ns("w_da2"):
            wait_buf(wd_v.at[pl.ds(*DA2)], sem_d.at[5])
        with ns("c_da2"):
            if not pure:
                finish(DA2[0], down(*DA2))
        with ns("w_da"):
            wait_buf(wd_v.at[pl.ds(*DA)], sem_d.at[0])
        with ns("c_da"):
            if not pure:
                finish(DA[0], down(*DA))
        with ns("w_db"):
            wait_buf(wd_v.at[pl.ds(*DB)], sem_d.at[1])
        with ns("c_db"):
            if not pure:
                finish(DB[0], down(*DB))
        with ns("w_e0"):
            wait_buf(wd_v.at[pl.ds(*DE0)], sem_d.at[2])
        with ns("c_e0"):
            if not pure:
                finish(DE0[0], down(*DE0))
        cs = esplit * CW
        with ns("w_e1"):
            wait_buf(wd_v.at[pl.ds(*DE1), pl.ds(0, cs)], sem_d.at[3])
        with ns("c_e1"):
            if not pure:
                y_s[...] = down(*DE1, 0, cs)
        with ns("w_e2"):
            wait_buf(wd_v.at[pl.ds(*DE1), pl.ds(cs, F - cs)], sem_d.at[4])
        with ns("c_e2"):
            if pure:
                o_ref[...] = jnp.zeros_like(o_ref)
            elif notail:
                finish(DE1[0], y_s[...])
            else:
                finish(DE1[0], y_s[...] + down(*DE1, cs, F))

    def fn(A_x, A_k_cache, A_v_cache, A_wq, A_wo, B_x, B_w_r, B_w_gate, B_w_up, B_w_down, c, w_mod):
        B, _, D = A_x.shape
        _, HKV, SK, DH = A_k_cache.shape
        W = min(4096, max(256, SK // 4))
        HD = A_wq.shape[1]
        F = B_w_gate.shape[1]
        hbm = pl.BlockSpec(memory_space=pltpu.HBM)
        blk = lambda w, p=P: w.reshape(p, D // p, w.shape[1])
        wbuf = lambda n: pltpu.VMEM((n // CW, P, D // P, CW), BF16)
        out = pl.pallas_call(
            kernel,
            out_shape=jax.ShapeDtypeStruct((B, D), A_x.dtype),
            in_specs=[hbm] * 11,
            out_specs=pl.BlockSpec(memory_space=pltpu.VMEM),
            scratch_shapes=[
                pltpu.VMEM((B, D), BF16), pltpu.VMEM((B, D), BF16), pltpu.VMEM((D,), BF16),
                pltpu.VMEM((3, PM, D // PM, 2 * D), BF16), wbuf(HD), wbuf(HD), wbuf(F), wbuf(F),
                pltpu.VMEM((D, F), BF16),
                pltpu.VMEM((G, 2, NH, W, DH), BF16),
                pltpu.VMEM((6, B, D), F32),
                pltpu.VMEM((HKV, 2 * B, DH), BF16), pltpu.VMEM((HKV, 2 * B, DH), F32),
                pltpu.VMEM((F // CW, B, CW), F32),
                pltpu.VMEM((2, B, D), F32),
                pltpu.VMEM((B, 64), F32),
                pltpu.SemaphoreType.DMA((5,)), pltpu.SemaphoreType.DMA((6,)), pltpu.SemaphoreType.DMA((G,)),
            ],
            compiler_params=pltpu.CompilerParams(vmem_limit_bytes=100 * 1024 * 1024,
                                                 disable_bounds_checks=nosc, disable_semaphore_checks=nosc),
        )(A_x.reshape(B, D), A_k_cache, A_v_cache, blk(A_wq), blk(A_wo.T), B_w_r, blk(B_w_gate), blk(B_w_up),
          B_w_down.T, c, blk(w_mod, PM))
        return out.reshape(B, 1, D)
    return fn


_impl = make(lead=4)


@jax.jit
def pallas_adaLN_cond__sliding_block_cached__moe_arch_mod__decode_kernel(
    A_x, A_k_cache, A_v_cache, A_wq, A_wo, B_x, B_w_r, B_w_gate, B_w_up, B_w_down, c, w_mod,
):
    return _impl(A_x, A_k_cache, A_v_cache, A_wq, A_wo, B_x, B_w_r, B_w_gate, B_w_up, B_w_down, c, w_mod)
```

```python
import jax
import jax.numpy as jnp
from jax import lax
from jax.experimental import pallas as pl
from jax.experimental.pallas import tpu as pltpu

F32 = jnp.float32
BF16 = jnp.bfloat16
NT = (((1,), (1,)), ((), ()))


def _layernorm(x):
    m = jnp.mean(x, axis=-1, keepdims=True)
    d = x - m
    v = jnp.mean(d * d, axis=-1, keepdims=True)
    return d / jnp.sqrt(v + 1e-5)


def make(rows=16, G=3, L=12, voff=0, nosc=True, lead=4, esplit=6, pure=False, notail=False, kq=1, dmode=0, scopes=False):
    import contextlib
    ns = (lambda n: jax.named_scope(n)) if scopes else (lambda n: contextlib.nullcontext())
    NH = 8
    CW = 512
    P = 4
    PM = 6

    def kernel(x_hbm, k_hbm, v_hbm, wq_hbm, wo_hbm, wr_hbm, wg_hbm, wu_hbm, wd_hbm, c_hbm, wm_hbm,
               o_ref,
               x_v, c_v, wr_v, wm_v, wq_v, wo_v, wg_v, wu_v, wd_v, kv_v, mod_s, q_s, o_s, act_s, fin_s, y_s,
               sem_w, sem_d, sem_kv):
        B, D = x_v.shape
        _, _, HG, SK, DH = k_hbm.shape
        HKV = NH * HG
        W = kv_v.shape[3]
        NG = B * HG
        NQ = wq_v.shape[0]
        NF = wg_v.shape[0]
        F = NF * CW
        S_X, S_M, S_Q, S_O, S_G = range(5)

        def small_copies():
            return [pltpu.make_async_copy(s, d, sem_w.at[S_X])
                    for s, d in ((c_hbm, c_v), (x_hbm, x_v), (wr_hbm, wr_v))]

        def copy_w(src, dst, j, blocks, r, sem, priority):
            cw = dst.shape[-1]
            pltpu.make_async_copy(src.at[blocks, pl.ds(r, 8), pl.ds(j * cw, cw)],
                                  dst.at[j, blocks, pl.ds(r, 8), :], sem).start(priority=priority)

        def wait_buf(buf, sem):
            pltpu.make_async_copy(buf, buf, sem).wait()

        def rows_loop(lo, hi, fn):
            def body(i, _):
                fn(pl.multiple_of(i * 8, 8))
                return 0
            lax.fori_loop(lo, hi, body, 0)

        def start_mod(lo, hi, p0):
            def step(r):
                for j in range(wm_v.shape[0]):
                    copy_w(wm_hbm, wm_v, j, pl.ds(0, PM // 2), r, sem_w.at[S_M], p0)
                    copy_w(wm_hbm, wm_v, j, pl.ds(PM // 2, PM // 2), r, sem_w.at[S_M], 1)
            rows_loop(lo, hi, step)

        def start_pair(a, b, lo, hi):
            def step(r):
                for j in range(a[1].shape[0]):
                    copy_w(a[0], a[1], j, pl.ds(0, P), r, sem_w.at[a[2]], 0)
                    copy_w(b[0], b[1], j, pl.ds(0, P), r, sem_w.at[b[2]], 1)
            rows_loop(lo, hi, step)

        def start_qo(u, n=1):
            start_pair((wq_hbm, wq_v, S_Q), (wo_hbm, wo_v, S_O), 2 * u, 2 * (u + n))

        def start_gu(lo, hi):
            start_pair((wg_hbm, wg_v, S_G), (wu_hbm, wu_v, S_G), lo, hi)

        DA, DA2, DB, DE0, DE1 = (0, 256), (448, 64), (256, 128), (384, 64), (512, 64)

        def copy_d(rng, r, j, sem, priority):
            r0, n = rng
            src = wd_hbm.at[pl.ds(r0, n)].reshape(P, n // P, F)
            dst = wd_v.at[pl.ds(r0, n)].reshape(P, n // P, F)
            pltpu.make_async_copy(src.at[:, pl.ds(r, 8), pl.ds(j * CW, CW)],
                                  dst.at[:, pl.ds(r, 8), pl.ds(j * CW, CW)], sem).start(priority=priority)

        def start_da(lo, hi, rng=DA, s=0):
            half = rng[1] // P // 2

            def step(r):
                for j in range(NF):
                    copy_d(rng, r, j, sem_d.at[s], 0)
                    copy_d(rng, pl.multiple_of(r + half, 8), j, sem_d.at[s], 1)
            rows_loop(lo, hi, step)

        def start_dlast(i):
            if dmode == 0:
                e_list = [(DE0, r, j, 2) for r in (0, 8) for j in range(NF)]
                e_list += [(DE1, r, j, 3) for r in (0, 8) for j in range(esplit)]
                e_list += [(DE1, r, j, 4) for r in (0, 8) for j in range(esplit, NF)]
            for j in range(NF):
                copy_d(DB, 8 * i, j, sem_d.at[1], 0)
                rng, r, jj, s = e_list[i * NF + j]
                copy_d(rng, r, jj, sem_d.at[s], 1)

        nr = W // rows
        part = nr // NH

        def start_kv(t):
            g = t // NH
            slot = g % G
            b = g // HG
            par = g % HG

            def body(i, _):
                for w, src in enumerate((k_hbm, v_hbm)):
                    r = pl.multiple_of(((i + w * voff) % nr) * rows, rows)
                    pltpu.make_async_copy(src.at[b, :, par, pl.ds(SK - W + r, rows), :],
                                          kv_v.at[slot, w, :, pl.ds(r, rows), :],
                                          sem_kv.at[slot]).start(priority=w ^ kq)
                return 0
            i0 = (t % NH) * part
            lax.fori_loop(0, part, lambda i, c: body(i0 + i, c), 0, unroll=2)

        def kv_loop(lo, hi):
            def body(t, _):
                start_kv(t)
                return 0
            lax.fori_loop(lo, hi, body, 0)

        if lead:
            start_mod(0, lead, 1)
        for cp in small_copies():
            cp.start(priority=1 if lead else 0)
        start_mod(lead, D // PM // 8, 0)
        start_qo(0, 4)
        for cp in small_copies():
            cp.wait()
        cf = c_v[...].astype(F32)
        sc = (cf * jax.nn.sigmoid(cf)).astype(BF16)
        wait_buf(wm_v, sem_w.at[S_M])

        def mod_step(j, _):
            if not pure:
                m = jnp.dot(sc, wm_v[j].reshape(D, 2 * D), preferred_element_type=F32)
                mod_s[2 * j] = m[:, :D]
                mod_s[2 * j + 1] = m[:, D:]
            start_qo(4 + j)
            return 0
        lax.fori_loop(0, 3, mod_step, 0)
        x = x_v[...].astype(F32)
        h = (_layernorm(x) * (1.0 + mod_s[1]) + mod_s[0]).astype(BF16)
        start_qo(7, 2)
        kv_loop(0, 4)
        wait_buf(wq_v, sem_w.at[S_Q])
        n_more = L - 4

        def q_step(j, _):
            if not pure:
                q = jnp.dot(h, wq_v[j].reshape(D, CW), preferred_element_type=F32)
                for i in range(2):
                    q2 = jnp.concatenate([q[:, (2 * i) * DH:(2 * i + 1) * DH],
                                          q[:, (2 * i + 1) * DH:(2 * i + 2) * DH]], axis=0)
                    q_s[2 * j + i] = q2.astype(BF16)
            kv_loop(4 + (j * n_more) // NQ, 4 + ((j + 1) * n_more) // NQ)
            return 0
        lax.fori_loop(0, NQ, q_step, 0)
        o_s[...] = jnp.zeros_like(o_s)

        scale = DH ** -0.5
        row_b = lax.broadcasted_iota(jnp.int32, (2 * B, DH), 0) % B
        NP = NG * NH

        def attend(t, _):
            g = t // NH
            j = t % NH
            slot = g % G
            b = g // HG
            hk = j * HG + g % HG

            @pl.when(j == 0)
            def _():
                wait_buf(kv_v.at[slot], sem_kv.at[slot])

            if not pure:
                s = lax.dot_general(q_s[hk], kv_v[slot, 0, j], NT, preferred_element_type=F32) * scale
                m = jnp.max(s, axis=-1, keepdims=True)
                p = jnp.exp(s - m)
                l = jnp.sum(p, axis=-1, keepdims=True)
                o = jnp.dot(p.astype(BF16), kv_v[slot, 1, j], preferred_element_type=F32) / l
                o_s[hk] = jnp.where(row_b == b, o, o_s[hk])
            u = t + L

            @pl.when(u < NP)
            def _():
                start_kv(u)

            @pl.when(u >= NP)
            def _():
                n2 = L - NH
                v = u - NP
                lo = jnp.where(v < n2, 2 * v, n2 + v)
                hi = jnp.where(v < n2, 2 * v + 2, n2 + v + 1)
                start_gu(lo, hi)
            return 0
        with ns('c_att'):
            lax.fori_loop(0, NP, attend, 0)
        g_done = 2 * (L - NH) + NH
        todo = [(lambda i=i: start_gu(i, i + 1)) for i in range(g_done, 18)]
        todo += [lambda: start_da(0, 1, DA2, 5)] + [(lambda i=i: start_da(i, i + 1)) for i in range(4)]

        wait_buf(wo_v, sem_w.at[S_O])

        def wo_step(j, acc):
            if not pure:
                o = jnp.concatenate([o_s[2 * j + i, k * B:(k + 1) * B, :] for i in range(2) for k in range(2)],
                                    axis=1).astype(BF16)
                acc = acc + lax.dot_general(o, wo_v[j].reshape(D, CW), NT, preferred_element_type=F32)

            for n in range(3):
                pl.when(j == 2 * n + 1)(todo[n])
            return acc
        with ns('c_wo'):
            attn = lax.fori_loop(0, NQ, wo_step, jnp.zeros((B, D), F32))
        todo[3]()
        x1 = x + mod_s[2] * attn
        h2 = _layernorm(x1) * (1.0 + mod_s[4]) + mod_s[3]
        r = jnp.sum(h2 * wr_v[...].astype(F32).reshape(1, D), axis=-1, keepdims=True)
        h2b = h2.astype(BF16)
        fin_s[0] = x1 + mod_s[5] * (h2 + h2 * 0.0)
        fin_s[1] = mod_s[5] * jax.nn.sigmoid(r)
        with ns("i_da"):
            for fn_ in todo[4:]:
                fn_()
            start_dlast(0)
        with ns("w_g"):
            wait_buf(wg_v, sem_w.at[S_G])
            wait_buf(wu_v, sem_w.at[S_G])

        def gu_step(j, _):
            if not pure:
                gate = jnp.dot(h2b, wg_v[j].reshape(D, CW), preferred_element_type=F32)
                up = jnp.dot(h2b, wu_v[j].reshape(D, CW), preferred_element_type=F32)
                act_s[j] = gate * jax.nn.sigmoid(gate) * up
            for i in range(1, 4):
                @pl.when(j == 2 * i - 1)
                def _():
                    start_dlast(i)
            return 0
        with ns('c_gu'):
            lax.fori_loop(0, NF, gu_step, 0)
        act = jnp.concatenate([act_s[j] for j in range(NF)], axis=1).astype(BF16)

        def down(r0, n, c0=0, c1=F):
            return lax.dot_general(act[:, c0:c1], wd_v[r0:r0 + n, c0:c1], NT, preferred_element_type=F32)

        def finish(r0, y):
            cs = slice(r0, r0 + y.shape[1])
            o_ref[:, cs] = (fin_s[0, :, cs] + fin_s[1, :, cs] * y).astype(o_ref.dtype)

        with ns("w_da2"):
            wait_buf(wd_v.at[pl.ds(*DA2)], sem_d.at[5])
        with ns("c_da2"):
            if not pure:
                finish(DA2[0], down(*DA2))
        with ns("w_da"):
            wait_buf(wd_v.at[pl.ds(*DA)], sem_d.at[0])
        with ns("c_da"):
            if not pure:
                finish(DA[0], down(*DA))
        with ns("w_db"):
            wait_buf(wd_v.at[pl.ds(*DB)], sem_d.at[1])
        with ns("c_db"):
            if not pure:
                finish(DB[0], down(*DB))
        with ns("w_e0"):
            wait_buf(wd_v.at[pl.ds(*DE0)], sem_d.at[2])
        with ns("c_e0"):
            if not pure:
                finish(DE0[0], down(*DE0))
        cs = esplit * CW
        with ns("w_e1"):
            wait_buf(wd_v.at[pl.ds(*DE1), pl.ds(0, cs)], sem_d.at[3])
        with ns("c_e1"):
            if not pure:
                y_s[...] = down(*DE1, 0, cs)
        with ns("w_e2"):
            wait_buf(wd_v.at[pl.ds(*DE1), pl.ds(cs, F - cs)], sem_d.at[4])
        with ns("c_e2"):
            if pure:
                o_ref[...] = jnp.zeros_like(o_ref)
            elif notail:
                finish(DE1[0], y_s[...])
            else:
                finish(DE1[0], y_s[...] + down(*DE1, cs, F))

    def fn(A_x, A_k_cache, A_v_cache, A_wq, A_wo, B_x, B_w_r, B_w_gate, B_w_up, B_w_down, c, w_mod):
        B, _, D = A_x.shape
        _, HKV, SK, DH = A_k_cache.shape
        W = min(4096, max(256, SK // 4))
        HD = A_wq.shape[1]
        F = B_w_gate.shape[1]
        hbm = pl.BlockSpec(memory_space=pltpu.HBM)
        blk = lambda w, p=P: w.reshape(p, D // p, w.shape[1])
        wbuf = lambda n: pltpu.VMEM((n // CW, P, D // P, CW), BF16)
        out = pl.pallas_call(
            kernel,
            out_shape=jax.ShapeDtypeStruct((B, D), A_x.dtype),
            in_specs=[hbm] * 11,
            out_specs=pl.BlockSpec(memory_space=pltpu.VMEM),
            scratch_shapes=[
                pltpu.VMEM((B, D), BF16), pltpu.VMEM((B, D), BF16), pltpu.VMEM((D,), BF16),
                pltpu.VMEM((3, PM, D // PM, 2 * D), BF16), wbuf(HD), wbuf(HD), wbuf(F), wbuf(F),
                pltpu.VMEM((D, F), BF16),
                pltpu.VMEM((G, 2, NH, W, DH), BF16),
                pltpu.VMEM((6, B, D), F32),
                pltpu.VMEM((HKV, 2 * B, DH), BF16), pltpu.VMEM((HKV, 2 * B, DH), F32),
                pltpu.VMEM((F // CW, B, CW), F32),
                pltpu.VMEM((2, B, D), F32),
                pltpu.VMEM((B, 64), F32),
                pltpu.SemaphoreType.DMA((5,)), pltpu.SemaphoreType.DMA((6,)), pltpu.SemaphoreType.DMA((G,)),
            ],
            compiler_params=pltpu.CompilerParams(vmem_limit_bytes=100 * 1024 * 1024,
                                                 disable_bounds_checks=nosc, disable_semaphore_checks=nosc),
        )(A_x.reshape(B, D), A_k_cache.reshape(B, NH, HKV // NH, SK, DH),
          A_v_cache.reshape(B, NH, HKV // NH, SK, DH), blk(A_wq), blk(A_wo.T), B_w_r, blk(B_w_gate), blk(B_w_up),
          B_w_down.T, c, blk(w_mod, PM))
        return out.reshape(B, 1, D)
    return fn


_impl = make()


@jax.jit
def pallas_adaLN_cond__sliding_block_cached__moe_arch_mod__decode_kernel(
    A_x, A_k_cache, A_v_cache, A_wq, A_wo, B_x, B_w_r, B_w_gate, B_w_up, B_w_down, c, w_mod,
):
    return _impl(A_x, A_k_cache, A_v_cache, A_wq, A_wo, B_x, B_w_r, B_w_gate, B_w_up, B_w_down, c, w_mod)
```

```python
import jax
import jax.numpy as jnp
from jax import lax
from jax.experimental import pallas as pl
from jax.experimental.pallas import tpu as pltpu

F32 = jnp.float32
BF16 = jnp.bfloat16
NT = (((1,), (1,)), ((), ()))

HEADS = 8
KV_ROWS = 16
SLOTS = 3
AHEAD = 12
LEAD = 5
BLOCKS = 4
COLS = 512
MOD_BLOCKS = 6
DOWN_ROWS = 16


def _layernorm(x):
    d = x - jnp.mean(x, axis=-1, keepdims=True)
    var = jnp.mean(d * d, axis=-1, keepdims=True)
    return d / jnp.sqrt(var + 1e-5)


def _silu(x):
    return x * jax.nn.sigmoid(x)


def _loop(lo, hi, body):
    def step(i, carry):
        body(i)
        return carry

    lax.fori_loop(lo, hi, step, 0)


def _wait(buf, sem):
    pltpu.make_async_copy(buf, buf, sem).wait()


def _kernel(
    x_hbm, c_hbm, wr_hbm, k_hbm, v_hbm, wm_hbm, wq_hbm, wo_hbm, wg_hbm, wu_hbm, wd_hbm,
    out_ref,
    x_v, c_v, wr_v, kv_v, wm_v, wq_v, wo_v, wg_v, wu_v, wd_v,
    mod_s, q_s, o_s, act_s, fin_s, y_s,
    sem_w, sem_d, sem_kv,
):
    batch, d_model = x_v.shape
    _, _, groups, cache_len, d_head = k_hbm.shape
    window = kv_v.shape[3]
    n_pairs = batch * groups * HEADS
    n_q, n_f = wq_v.shape[0], wg_v.shape[0]
    d_ff = n_f * COLS
    row_steps = d_model // BLOCKS // 8
    sem_small, sem_m, sem_q, sem_o, sem_g = (sem_w.at[i] for i in range(5))

    def copy_chunk(src, dst, chunk, blocks, step, sem, queue):
        rows = pl.ds(pl.multiple_of(step * 8, 8), 8)
        cols = dst.shape[-1]
        pltpu.make_async_copy(
            src.at[blocks, rows, pl.ds(chunk * cols, cols)], dst.at[chunk, blocks, rows, :], sem
        ).start(priority=queue)

    def small_copies():
        pairs = ((c_hbm, c_v), (x_hbm, x_v), (wr_hbm, wr_v))
        return [pltpu.make_async_copy(src, dst, sem_small) for src, dst in pairs]

    def start_mod(lo, hi, first_queue):
        half = MOD_BLOCKS // 2

        def step(i):
            for j in range(wm_v.shape[0]):
                copy_chunk(wm_hbm, wm_v, j, pl.ds(0, half), i, sem_m, first_queue)
                copy_chunk(wm_hbm, wm_v, j, pl.ds(half, half), i, sem_m, 1)

        _loop(lo, hi, step)

    def start_two(first, second, lo, hi):
        def step(i):
            for j in range(first[1].shape[0]):
                for queue, (src, dst, sem) in enumerate((first, second)):
                    copy_chunk(src, dst, j, pl.ds(0, BLOCKS), i, sem, queue)

        _loop(lo, hi, step)

    def start_qo(lo, hi):
        start_two((wq_hbm, wq_v, sem_q), (wo_hbm, wo_v, sem_o), lo, hi)

    def start_gu(lo, hi):
        start_two((wg_hbm, wg_v, sem_g), (wu_hbm, wu_v, sem_g), lo, hi)

    def start_kv(unit):
        group = unit // HEADS
        slot = group % SLOTS
        steps = window // KV_ROWS // HEADS

        def step(i):
            row = pl.multiple_of(((unit % HEADS) * steps + i) * KV_ROWS, KV_ROWS)
            for which, src in enumerate((k_hbm, v_hbm)):
                pltpu.make_async_copy(
                    src.at[group // groups, :, group % groups,
                           pl.ds(cache_len - window + row, KV_ROWS), :],
                    kv_v.at[slot, which, :, pl.ds(row, KV_ROWS), :],
                    sem_kv.at[slot],
                ).start(priority=1 - which)

        _loop(0, steps, step)

    def copy_down(rng, step, chunk, sem, queue):
        idx = (pl.ds(rng * BLOCKS, BLOCKS), pl.ds(pl.multiple_of(step * 8, 8), 8),
               pl.ds(chunk * COLS, COLS))
        pltpu.make_async_copy(wd_hbm.at[idx], wd_v.at[idx], sem_d.at[sem]).start(priority=queue)

    def start_down(rng, sem):
        for j in range(n_f):
            copy_down(rng, 0, j, sem, 0)
            copy_down(rng, 1, j, sem, 1)

    split = 2 * n_f // 3
    last = [(6, i, j, 3) for i in range(2) for j in range(n_f)]
    last += [(8, i, j, 4) for i in range(2) for j in range(split)]
    last += [(8, i, j, 5) for i in range(2) for j in range(split, n_f)]

    def start_down_last(part):
        for j in range(n_f):
            copy_down(4 + part // 2, part % 2, j, 2, 0)
            copy_down(*last[part * n_f + j], 1)

    start_mod(0, LEAD, 1)
    for copy in small_copies():
        copy.start(priority=1)
    start_mod(LEAD, d_model // MOD_BLOCKS // 8, 0)
    start_qo(0, 8)
    for copy in small_copies():
        copy.wait()
    cond = _silu(c_v[...].astype(F32)).astype(BF16)
    _wait(wm_v, sem_m)

    def mod_step(j):
        m = jnp.dot(cond, wm_v[j].reshape(d_model, 2 * d_model), preferred_element_type=F32)
        mod_s[2 * j] = m[:, :d_model]
        mod_s[2 * j + 1] = m[:, d_model:]
        start_qo(8 + 2 * j, 10 + 2 * j)

    _loop(0, 3, mod_step)
    shift_a, scale_a, gate_a, shift_b, scale_b, gate_b = range(6)
    x = x_v[...].astype(F32)
    h = (_layernorm(x) * (1.0 + mod_s[scale_a]) + mod_s[shift_a]).astype(BF16)
    start_qo(14, row_steps)
    _loop(0, 4, start_kv)
    _wait(wq_v, sem_q)
    per_chunk = COLS // d_head // 2

    def q_step(j):
        q = jnp.dot(h, wq_v[j].reshape(d_model, COLS), preferred_element_type=F32)
        for i in range(per_chunk):
            heads = [q[:, (2 * i + k) * d_head:(2 * i + k + 1) * d_head] for k in range(2)]
            q_s[per_chunk * j + i] = jnp.concatenate(heads, axis=0).astype(BF16)
        _loop(4 + j * (AHEAD - 4) // n_q, 4 + (j + 1) * (AHEAD - 4) // n_q, start_kv)

    _loop(0, n_q, q_step)
    o_s[...] = jnp.zeros_like(o_s)

    row_batch = lax.broadcasted_iota(jnp.int32, (2 * batch, d_head), 0) % batch
    early = AHEAD - HEADS

    def attend(t):
        group, j = t // HEADS, t % HEADS
        slot = group % SLOTS
        head = j * groups + group % groups

        @pl.when(j == 0)
        def _():
            _wait(kv_v.at[slot], sem_kv.at[slot])

        s = lax.dot_general(q_s[head], kv_v[slot, 0, j], NT, preferred_element_type=F32)
        s = s * d_head**-0.5
        p = jnp.exp(s - jnp.max(s, axis=-1, keepdims=True))
        o = jnp.dot(p.astype(BF16), kv_v[slot, 1, j], preferred_element_type=F32)
        o = o / jnp.sum(p, axis=-1, keepdims=True)
        o_s[head] = jnp.where(row_batch == group // groups, o, o_s[head])

        unit = t + AHEAD

        @pl.when(unit < n_pairs)
        def _():
            start_kv(unit)

        @pl.when(unit >= n_pairs)
        def _():
            n = unit - n_pairs
            start_gu(jnp.where(n < early, 2 * n, early + n),
                     jnp.where(n < early, 2 * n + 2, early + n + 1))

    _loop(0, n_pairs, attend)
    gu_done = 2 * early + HEADS

    _wait(wo_v, sem_o)

    def wo_step(j, acc):
        o = jnp.concatenate(
            [o_s[per_chunk * j + i, k * batch:(k + 1) * batch, :]
             for i in range(per_chunk) for k in range(2)], axis=1)
        acc += lax.dot_general(o.astype(BF16), wo_v[j].reshape(d_model, COLS), NT,
                               preferred_element_type=F32)

        @pl.when((j == 1) | (j == 3))
        def _():
            start_gu(gu_done + j // 2, gu_done + j // 2 + 1)

        @pl.when(j == 5)
        def _():
            start_down(7, 0)

        return acc

    attn = lax.fori_loop(0, n_q, wo_step, jnp.zeros((batch, d_model), F32))
    start_down(0, 1)
    x1 = x + mod_s[gate_a] * attn
    h2 = _layernorm(x1) * (1.0 + mod_s[scale_b]) + mod_s[shift_b]
    r = jnp.sum(h2 * wr_v[...].astype(F32).reshape(1, d_model), axis=-1, keepdims=True)
    fin_s[0] = x1 + mod_s[gate_b] * (h2 + h2 * 0.0)
    fin_s[1] = mod_s[gate_b] * jax.nn.sigmoid(r)
    h2 = h2.astype(BF16)
    _loop(1, 4, lambda rng: start_down(rng, 1))

    _wait(wg_v, sem_g)
    _wait(wu_v, sem_g)

    def gu_step(j):
        gate = jnp.dot(h2, wg_v[j].reshape(d_model, COLS), preferred_element_type=F32)
        up = jnp.dot(h2, wu_v[j].reshape(d_model, COLS), preferred_element_type=F32)
        act_s[j] = _silu(gate) * up
        for part in range(1, 4):
            pl.when(j == 2 * part - 1)(lambda part=part: start_down_last(part))

    start_down_last(0)
    _loop(0, n_f, gu_step)
    act = jnp.concatenate([act_s[j] for j in range(n_f)], axis=1).astype(BF16)
    rng_rows = BLOCKS * DOWN_ROWS

    def wait_down(rng, n, sem, c0=0, c1=d_ff):
        _wait(wd_v.at[pl.ds(rng * BLOCKS, n * BLOCKS), :, pl.ds(c0, c1 - c0)], sem_d.at[sem])

    def down(rng, n, c0=0, c1=d_ff):
        w = wd_v[rng * BLOCKS:(rng + n) * BLOCKS, :, c0:c1].reshape(n * rng_rows, c1 - c0)
        return lax.dot_general(act[:, c0:c1], w, NT, preferred_element_type=F32)

    def finish(rng, y):
        cols = slice(rng * rng_rows, rng * rng_rows + y.shape[1])
        out_ref[:, cols] = (fin_s[0, :, cols] + fin_s[1, :, cols] * y).astype(out_ref.dtype)

    for sem, (rng, n) in enumerate(((7, 1), (0, 4), (4, 2), (6, 1))):
        wait_down(rng, n, sem)
        finish(rng, down(rng, n))
    wait_down(8, 1, 4, 0, split * COLS)
    y_s[...] = down(8, 1, 0, split * COLS)
    wait_down(8, 1, 5, split * COLS)
    finish(8, y_s[...] + down(8, 1, split * COLS))


@jax.jit
def pallas_adaLN_cond__sliding_block_cached__moe_arch_mod__decode_kernel(
    A_x: jax.Array,
    A_k_cache: jax.Array,
    A_v_cache: jax.Array,
    A_wq: jax.Array,
    A_wo: jax.Array,
    B_x: jax.Array,
    B_w_r: jax.Array,
    B_w_gate: jax.Array,
    B_w_up: jax.Array,
    B_w_down: jax.Array,
    c: jax.Array,
    w_mod: jax.Array,
):
    del B_x
    batch, seq, d_model = A_x.shape
    _, kv_heads, cache_len, d_head = A_k_cache.shape
    window = min(4096, max(256, cache_len // 4))
    d_attn, d_ff = A_wq.shape[1], B_w_gate.shape[1]
    assert seq == 1 and d_attn == 2 * kv_heads * d_head
    assert (d_model, d_attn, d_ff) == (576, 4096, 4608)

    def heads(cache):
        return cache.reshape(batch, HEADS, kv_heads // HEADS, cache_len, d_head)

    def row_blocks(w, n=BLOCKS):
        return w.reshape(n, d_model // n, w.shape[1])

    def chunked(cols):
        return pltpu.VMEM((cols // COLS, BLOCKS, d_model // BLOCKS, COLS), BF16)

    out = pl.pallas_call(
        _kernel,
        out_shape=jax.ShapeDtypeStruct((batch, d_model), A_x.dtype),
        in_specs=[pl.BlockSpec(memory_space=pltpu.HBM)] * 11,
        out_specs=pl.BlockSpec(memory_space=pltpu.VMEM),
        scratch_shapes=[
            pltpu.VMEM((batch, d_model), BF16),
            pltpu.VMEM((batch, d_model), BF16),
            pltpu.VMEM((d_model,), BF16),
            pltpu.VMEM((SLOTS, 2, HEADS, window, d_head), BF16),
            pltpu.VMEM((3, MOD_BLOCKS, d_model // MOD_BLOCKS, 2 * d_model), BF16),
            chunked(d_attn),
            chunked(d_attn),
            chunked(d_ff),
            chunked(d_ff),
            pltpu.VMEM((d_model // DOWN_ROWS, DOWN_ROWS, d_ff), BF16),
            pltpu.VMEM((6, batch, d_model), F32),
            pltpu.VMEM((kv_heads, 2 * batch, d_head), BF16),
            pltpu.VMEM((kv_heads, 2 * batch, d_head), F32),
            pltpu.VMEM((d_ff // COLS, batch, COLS), F32),
            pltpu.VMEM((2, batch, d_model), F32),
            pltpu.VMEM((batch, BLOCKS * DOWN_ROWS), F32),
            pltpu.SemaphoreType.DMA((5,)),
            pltpu.SemaphoreType.DMA((6,)),
            pltpu.SemaphoreType.DMA((SLOTS,)),
        ],
        compiler_params=pltpu.CompilerParams(
            vmem_limit_bytes=80 * 1024 * 1024, disable_semaphore_checks=True
        ),
    )(
        A_x.reshape(batch, d_model),
        c,
        B_w_r,
        heads(A_k_cache),
        heads(A_v_cache),
        row_blocks(w_mod, MOD_BLOCKS),
        row_blocks(A_wq),
        row_blocks(A_wo.T),
        row_blocks(B_w_gate),
        row_blocks(B_w_up),
        row_blocks(B_w_down.T, d_model // DOWN_ROWS),
    )
    return out.reshape(batch, seq, d_model)
```
